```python
import os as _os
_os.environ.setdefault("JAX_PLATFORMS", "cpu")
import jax
import jax.numpy as jnp

def _softmax(x, axis=-1):
    return jax.nn.softmax(x, axis=axis)
def _gelu(x):
    return jax.nn.gelu(x, approximate=True)
def _silu(x):
    return jax.nn.silu(x)
def _sigmoid(x):
    return jax.nn.sigmoid(x)
def _layernorm(x, axis=-1, eps=1e-5):
    m = jnp.mean(x, axis=axis, keepdims=True)
    v = jnp.var(x, axis=axis, keepdims=True)
    return (x - m) / jnp.sqrt(v + eps)
def _scatter_add(tgt, idx, src, axis=0):
    return tgt.at[idx].add(src)
def _segment_sum(src, seg, n):
    return jax.ops.segment_sum(src, seg, n)
class _Rng:
    def __init__(self, key):
        self._k = key
    def _next(self):
        self._k, sub = jax.random.split(self._k)
        return sub
    def normal(self, shape):
        return jax.random.normal(self._next(), shape, dtype=jnp.bfloat16)
    def randint(self, lo, hi, shape):
        return jax.random.randint(self._next(), shape, lo, hi, dtype=jnp.int32)
    def uniform(self, shape, lo=0.0, hi=1.0):
        return jax.random.uniform(self._next(), shape, jnp.bfloat16, lo, hi)
    def permutation(self, n):
        return jax.random.permutation(self._next(), n)


kernel_name = 'standalone__mha_softmax__near_ridge'

def setup_inputs():
    _rng = _Rng(jax.random.key(int.from_bytes(__import__("os").urandom(4), "little")))
    _w = (lambda a: (lambda t: t.astype(jnp.bfloat16) if jnp.issubdtype(t.dtype, jnp.floating) else t)(jnp.asarray(a)))
    B, H, Sq, Sk, D = 8, 32, 496, 512, 192
    return {
        "q": _w((lambda *s: _rng.normal(s) * 0.05)(B, H, Sq, D)),
        "k": _w((lambda *s: _rng.normal(s) * 3.2)(B, H, Sk, D)),
        "v": _w((lambda *s: _rng.normal(s) * 0.05)(B, H, Sk, D)),
    }

def reference(q, k, v):
    scale = q.shape[-1] ** -0.5
    scores = jnp.einsum("bhqd,bhkd->bhqk", q, k) * scale
    p = _softmax(scores, axis=-1)
    return jnp.einsum("bhqk,bhkd->bhqd", p, v)
```

```python
import jax
import jax.numpy as jnp
from jax import lax
import jax.experimental.pallas as pl
import jax.experimental.pallas.tpu as pltpu

_LOG2E = 1.4426950408889634
_U = 32
_R = 8
_W = 256
_NB = 3


def _mha_kernel(qt_hbm, kt_hbm, vt_hbm, ot_hbm, qo, kv, p_scr, q_scr, sq, skv, so):
    nh, d, sq_len = qt_hbm.shape
    n_it = nh // _U
    c = d ** -0.5 * _LOG2E
    qb, ob = qo.at[0], qo.at[1]

    def copy_q(h, s):
        return pltpu.make_async_copy(qt_hbm.at[h], qb.at[s], sq.at[s])

    def copy_k(h, s):
        return pltpu.make_async_copy(kt_hbm.at[h], kv.at[s, 0], skv.at[s])

    def copy_v(h, s):
        return pltpu.make_async_copy(vt_hbm.at[h], kv.at[s, 1], skv.at[s])

    def copy_o(h, s):
        return pltpu.make_async_copy(ob.at[s], ot_hbm.at[h], so.at[s])

    def wait_kv(s):
        pltpu.make_async_copy(kv.at[s], kv.at[s], skv.at[s]).wait()

    def fill(s, carry):
        copy_q(s, s).start()
        copy_k(s, s).start()
        copy_v(s, s).start()
        return carry

    lax.fori_loop(0, _R, fill, 0)
    copy_q(0, 0).wait()
    q_scr[...] = qb[0].T
    wait_kv(0)

    chunks = [(g, j, min(_W, sq_len - j))
              for g in range(_U) for j in range(0, sq_len, _W)]
    n = len(chunks)

    def body(it, carry):
        h0 = it * _U
        more = it < n_it - 1

        def if_exists(g, fn):
            if g < _U:
                fn()
            else:
                pl.when(more)(fn)

        def refill(copy, g):
            if_exists(g + _R, lambda: copy(h0 + g + _R, g % _R).start())

        q_rows = {}

        def stage_a(t):
            g, j, w = chunks[t]
            s = g % _R
            if g not in q_rows:
                q_rows[g] = q_scr[...] if g == 0 else qb[s].T
            sc = jnp.dot(q_rows[g][j:j + w], kv[s, 0],
                         preferred_element_type=jnp.float32)
            if j + w == sq_len:
                refill(copy_q, g)
                refill(copy_k, g)
                g1 = g + 1
                if_exists(g1, lambda: wait_kv(g1 % _R))
                if_exists(g1, lambda: copy_q(h0 + g1, g1 % _R).wait())
                if g1 >= _R:
                    copy_o(h0 + g1 - _R, g1 % _R).wait()
                else:
                    pl.when(it > 0)(lambda: copy_o(h0 + g1 - _R, g1 % _R).wait())
            return sc, jnp.max(sc, axis=1, keepdims=True)

        def stage_b(t, sc, m):
            w = chunks[t][2]
            p = jnp.exp2((sc - m) * c)
            l = jnp.sum(p, axis=1, keepdims=True)
            lb = jnp.broadcast_to(l, (w, 128))
            eye = (lax.broadcasted_iota(jnp.int32, (128, 128), 0)
                   == lax.broadcasted_iota(jnp.int32, (128, 128), 1))
            parts = []
            for r0 in range(0, w, 128):
                rows = min(128, w - r0)
                diag = jnp.where(eye[:rows], lb[r0:r0 + rows], 0.0)
                parts.append(jnp.sum(diag, axis=0, keepdims=True))
            p_scr[t % _NB][:w, :] = p.astype(jnp.bfloat16)
            return jnp.concatenate(parts, axis=1)[:, :w]

        def stage_c(t, l_row):
            g, j, w = chunks[t]
            s = g % _R
            ot = lax.dot_general(kv[s, 1], p_scr[t % _NB][:w, :],
                                 (((1,), (1,)), ((), ())),
                                 preferred_element_type=jnp.float32)
            ob[s, :, j:j + w] = (ot * (1.0 / l_row)).astype(ob.dtype)
            if j + w == sq_len:
                refill(copy_v, g)
                copy_o(h0 + g, s).start()

        scores, sums = {}, {}
        for t in range(-1, n + 1):
            if t + 1 < n:
                scores[t + 1] = stage_a(t + 1)
            if 0 <= t < n:
                sums[t] = stage_b(t, *scores.pop(t))
            if t >= 1:
                stage_c(t - 1, sums.pop(t - 1))
            if t == n - 2:
                q_scr[...] = qb[0].T
        return carry

    lax.fori_loop(0, n_it, body, 0)
    for g in range(_U - _R + 1, _U):
        copy_o(nh - _U + g, g % _R).wait()


@jax.jit
def pallas_standalone__mha_softmax__near_ridge_kernel(
    q: jax.Array,
    k: jax.Array,
    v: jax.Array,
):
    b, h, sq_len, d = q.shape
    sk_len = k.shape[2]
    nh = b * h
    assert nh % _U == 0
    qt = jnp.swapaxes(q, 2, 3).reshape(nh, d, sq_len)
    kt = jnp.swapaxes(k, 2, 3).reshape(nh, d, sk_len)
    vt = jnp.swapaxes(v, 2, 3).reshape(nh, d, sk_len)
    any_spec = pl.BlockSpec(memory_space=pl.ANY)
    ot = pl.pallas_call(
        _mha_kernel,
        in_specs=[any_spec, any_spec, any_spec],
        out_specs=any_spec,
        out_shape=jax.ShapeDtypeStruct((nh, d, sq_len), q.dtype),
        scratch_shapes=[
            pltpu.VMEM((2, _R, d, sq_len), q.dtype),
            pltpu.VMEM((_R, 2, d, sk_len), k.dtype),
            [pltpu.VMEM((_W, sk_len), jnp.bfloat16) for _ in range(_NB)],
            pltpu.VMEM((sq_len, d), q.dtype),
            pltpu.SemaphoreType.DMA((_R,)),
            pltpu.SemaphoreType.DMA((_R,)),
            pltpu.SemaphoreType.DMA((_R,)),
        ],
        compiler_params=pltpu.CompilerParams(
            vmem_limit_bytes=64 * 1024 * 1024,
            flags={"XLA_TPU_RESCHEDULE_DMA_DONES": True},
        ),
    )(qt, kt, vt)
    return jnp.swapaxes(ot.reshape(b, h, d, sq_len), 2, 3)
```

```python
import jax
import jax.numpy as jnp
from jax import lax
import jax.experimental.pallas as pl
import jax.experimental.pallas.tpu as pltpu

_LOG2E = 1.4426950408889634
_U = 32
_R = 4
_W = 256
_NB = 3


def _mha_kernel(qt_hbm, kt_hbm, vt_hbm, ot_hbm, qo, kv, p_scr, q_scr,
                sem_q, sem_k, sem_v, sem_o):
    nh, d, sq_len = qt_hbm.shape
    n_it = nh // _U
    c = d ** -0.5 * _LOG2E
    qb, ob = qo.at[0], qo.at[1]

    def copy_q(h, s):
        return pltpu.make_async_copy(qt_hbm.at[h], qb.at[s], sem_q.at[s])

    def copy_k(h, s):
        return pltpu.make_async_copy(kt_hbm.at[h], kv.at[s, 0], sem_k.at[s])

    def copy_v(h, s):
        return pltpu.make_async_copy(vt_hbm.at[h], kv.at[s, 1], sem_v.at[s])

    def copy_o(h, s):
        return pltpu.make_async_copy(ob.at[s], ot_hbm.at[h], sem_o.at[s])

    def fill(s, carry):
        copy_q(s, s).start()
        copy_k(s, s).start()
        copy_v(s, s).start()
        return carry

    lax.fori_loop(0, _R, fill, 0)
    copy_q(0, 0).wait()
    q_scr[...] = qb[0].T
    copy_k(0, 0).wait()

    chunks = [(g, j, min(_W, sq_len - j))
              for g in range(_U) for j in range(0, sq_len, _W)]
    n = len(chunks)

    def body(it, carry):
        h0 = it * _U
        more = it < n_it - 1

        def if_exists(g, fn):
            if g < _U:
                fn()
            else:
                pl.when(more)(fn)

        def refill(copy, g):
            if_exists(g + _R, lambda: copy(h0 + g + _R, g % _R).start())

        q_rows = {}

        def stage_a(t):
            g, j, w = chunks[t]
            s = g % _R
            if g not in q_rows:
                q_rows[g] = q_scr[...] if g == 0 else qb[s].T
            sc = jnp.dot(q_rows[g][j:j + w], kv[s, 0],
                         preferred_element_type=jnp.float32)
            if j + w == sq_len:
                refill(copy_q, g)
                refill(copy_k, g)
                g1 = g + 1
                if_exists(g1, lambda: copy_k(h0 + g1, g1 % _R).wait())
                if_exists(g1, lambda: copy_q(h0 + g1, g1 % _R).wait())
                copy_v(h0 + g, s).wait()
                if g1 >= _R:
                    copy_o(h0 + g1 - _R, g1 % _R).wait()
                else:
                    pl.when(it > 0)(lambda: copy_o(h0 + g1 - _R, g1 % _R).wait())
            return sc, jnp.max(sc, axis=1, keepdims=True)

        def stage_b(t, sc, m):
            w = chunks[t][2]
            p = jnp.exp2((sc - m) * c)
            l = jnp.sum(p, axis=1, keepdims=True)
            lb = jnp.broadcast_to(l, (w, 128))
            eye = (lax.broadcasted_iota(jnp.int32, (128, 128), 0)
                   == lax.broadcasted_iota(jnp.int32, (128, 128), 1))
            parts = []
            for r0 in range(0, w, 128):
                rows = min(128, w - r0)
                diag = jnp.where(eye[:rows], lb[r0:r0 + rows], 0.0)
                parts.append(jnp.sum(diag, axis=0, keepdims=True))
            p_scr[t % _NB][:w, :] = p.astype(jnp.bfloat16)
            return jnp.concatenate(parts, axis=1)[:, :w]

        def stage_c(t, l_row):
            g, j, w = chunks[t]
            s = g % _R
            ot = lax.dot_general(kv[s, 1], p_scr[t % _NB][:w, :],
                                 (((1,), (1,)), ((), ())),
                                 preferred_element_type=jnp.float32)
            ob[s, :, j:j + w] = (ot * (1.0 / l_row)).astype(ob.dtype)
            if j + w == sq_len:
                refill(copy_v, g)
                copy_o(h0 + g, s).start()

        scores, sums = {}, {}
        for t in range(-1, n + 1):
            if t + 1 < n:
                scores[t + 1] = stage_a(t + 1)
            if 0 <= t < n:
                sums[t] = stage_b(t, *scores.pop(t))
            if t >= 1:
                stage_c(t - 1, sums.pop(t - 1))
            if t == n - 2:
                q_scr[...] = qb[0].T
        return carry

    lax.fori_loop(0, n_it, body, 0)
    for g in range(_U - _R + 1, _U):
        copy_o(nh - _U + g, g % _R).wait()


@jax.jit
def pallas_standalone__mha_softmax__near_ridge_kernel(
    q: jax.Array,
    k: jax.Array,
    v: jax.Array,
):
    b, h, sq_len, d = q.shape
    sk_len = k.shape[2]
    nh = b * h
    assert nh % _U == 0 and _U % _R == 0
    qt = jnp.swapaxes(q, 2, 3).reshape(nh, d, sq_len)
    kt = jnp.swapaxes(k, 2, 3).reshape(nh, d, sk_len)
    vt = jnp.swapaxes(v, 2, 3).reshape(nh, d, sk_len)
    any_spec = pl.BlockSpec(memory_space=pl.ANY)
    ot = pl.pallas_call(
        _mha_kernel,
        in_specs=[any_spec, any_spec, any_spec],
        out_specs=any_spec,
        out_shape=jax.ShapeDtypeStruct((nh, d, sq_len), q.dtype),
        scratch_shapes=[
            pltpu.VMEM((2, _R, d, sq_len), q.dtype),
            pltpu.VMEM((_R, 2, d, sk_len), k.dtype),
            [pltpu.VMEM((_W, sk_len), jnp.bfloat16) for _ in range(_NB)],
            pltpu.VMEM((sq_len, d), q.dtype),
            pltpu.SemaphoreType.DMA((_R,)),
            pltpu.SemaphoreType.DMA((_R,)),
            pltpu.SemaphoreType.DMA((_R,)),
            pltpu.SemaphoreType.DMA((_R,)),
        ],
        compiler_params=pltpu.CompilerParams(
            vmem_limit_bytes=64 * 1024 * 1024,
            flags={"XLA_TPU_RESCHEDULE_DMA_DONES": True},
        ),
    )(qt, kt, vt)
    return jnp.swapaxes(ot.reshape(b, h, d, sq_len), 2, 3)
```
